```python
import jax
import jax.numpy as jnp

def _softmax(x, axis=-1):
    return jax.nn.softmax(x, axis=axis)

def _gelu(x):
    return jax.nn.gelu(x, approximate=True)

def _silu(x):
    return jax.nn.silu(x)

def _sigmoid(x):
    return jax.nn.sigmoid(x)

def _layernorm(x, axis=-1, eps=1e-05):
    m = jnp.mean(x, axis=axis, keepdims=True)
    v = jnp.var(x, axis=axis, keepdims=True)
    return (x - m) / jnp.sqrt(v + eps)

def _scatter_add(tgt, idx, src, axis=0):
    return tgt.at[idx].add(src)

def _segment_sum(src, seg, n):
    return jax.ops.segment_sum(src, seg, n)

class _Rng:

    def __init__(self, key):
        self._k = key

    def _next(self):
        self._k, sub = jax.random.split(self._k)
        return sub

    def normal(self, shape):
        return jax.random.normal(self._next(), shape, dtype=jnp.bfloat16)

    def randint(self, lo, hi, shape):
        return jax.random.randint(self._next(), shape, lo, hi, dtype=jnp.int32)

    def uniform(self, shape, lo=0.0, hi=1.0):
        return jax.random.uniform(self._next(), shape, jnp.bfloat16, lo, hi)

    def permutation(self, n):
        return jax.random.permutation(self._next(), n)
kernel_name = 'interleave_layers__memory_aug_infini_attn__mixer_s_mlp__prompt'

def setup_inputs():
    _rng = _Rng(jax.random.key(int.from_bytes(__import__("os").urandom(4), "little")))
    _w = lambda a: (lambda t: t.astype(jnp.bfloat16) if jnp.issubdtype(t.dtype, jnp.floating) else t)(jnp.asarray(a))

    def _A_setup():
        B, S, D, H = (1, 2048, 1024, 32)
        N = 4
        L = max(1, S // N)
        sc = D ** (-0.5)
        return {'x': _w((lambda *s: _rng.normal(s) * 0.05)(B, N * L, D)), 'wq': _w((lambda *s: _rng.normal(s) * 0.05)(D, D) * sc), 'wk': _w((lambda *s: _rng.normal(s) * 0.05)(D, D) * sc), 'wv': _w((lambda *s: _rng.normal(s) * 0.05)(D, D) * sc), 'wo': _w((lambda *s: _rng.normal(s) * 0.05)(D, D) * sc), 'beta': _w((lambda *s: _rng.normal(s) * 0.05)(H))}
    _A_in = _A_setup()

    def _B_setup():
        B, S, D, F = (1, 2048, 1024, 3584)
        return {'x': _w((lambda *s: _rng.normal(s) * 0.05)(B, S, D)), 'w1': _w((lambda *s: _rng.normal(s) * 0.05)(D, D) * D ** (-0.5)), 'w2': _w((lambda *s: _rng.normal(s) * 0.05)(D, D) * D ** (-0.5)), 'w3': _w((lambda *s: _rng.normal(s) * 0.05)(D, F) * D ** (-0.5)), 'w4': _w((lambda *s: _rng.normal(s) * 0.05)(F, D) * F ** (-0.5))}
    _B_in = _B_setup()
    return {'A_x': _A_in['x'], 'A_wq': _A_in['wq'], 'A_wk': _A_in['wk'], 'A_wv': _A_in['wv'], 'A_wo': _A_in['wo'], 'A_beta': _A_in['beta'], 'B_x': _B_in['x'], 'B_w1': _B_in['w1'], 'B_w2': _B_in['w2'], 'B_w3': _B_in['w3'], 'B_w4': _B_in['w4']}

def reference(A_x, A_wq, A_wk, A_wv, A_wo, A_beta, B_x, B_w1, B_w2, B_w3, B_w4):

    def _A_ref(x, wq, wk, wv, wo, beta):
        B, S, D = x.shape
        H = 32
        Dh = D // H
        N = 4
        L = S // N
        q = (lambda x, *d: x.transpose(*d))((x @ wq).reshape(B, S, H, Dh), 0, 2, 1, 3).reshape(B, H, N, L, Dh)
        k = (lambda x, *d: x.transpose(*d))((x @ wk).reshape(B, S, H, Dh), 0, 2, 1, 3).reshape(B, H, N, L, Dh)
        v = (lambda x, *d: x.transpose(*d))((x @ wv).reshape(B, S, H, Dh), 0, 2, 1, 3).reshape(B, H, N, L, Dh)
        phi = lambda t: jnp.where(t > 0, t + 1.0, jnp.exp(t))
        scale = Dh ** (-0.5)
        ar = jnp.arange(L)
        mask = (lambda x, dt: x.astype(dt))(ar[:, None] < ar[None, :], x.dtype) * -1000000000.0
        g = _sigmoid(beta).reshape(1, H, 1, 1)
        M = jnp.einsum('bhd,bhe->bhde', q[:, :, 0, 0, :] * 0.0, q[:, :, 0, 0, :] * 0.0)
        z = q[:, :, 0, 0, :] * 0.0
        outs = []
        for s in range(N):
            qs, ks, vs = (q[:, :, s].copy(), k[:, :, s].copy(), v[:, :, s].copy())
            logits = jnp.einsum('bhqd,bhkd->bhqk', qs, ks) * scale + mask
            p = _softmax(logits, axis=-1)
            a_dot = jnp.einsum('bhqk,bhkd->bhqd', p, vs)
            pq = phi(qs)
            num = jnp.einsum('bhld,bhde->bhle', pq, M)
            den = jnp.einsum('bhld,bhd->bhl', pq, z)[..., None] + 1e-06
            a_mem = num / den
            o = g * a_mem + (1.0 - g) * a_dot
            outs.append(o)
            pk = phi(ks)
            M = M + jnp.einsum('bhld,bhle->bhde', pk, vs)
            z = z + jnp.einsum('bhld->bhd', pk)
        o = (lambda x, *d: x.transpose(*d))(jnp.stack(outs, 2).reshape(B, H, S, Dh), 0, 2, 1, 3).reshape(B, S, D)
        return o @ wo

    def _B_ref(x, w1, w2, w3, w4):
        B, S, D = x.shape
        h = _gelu(_layernorm(x, axis=-1) @ w1)
        c = D // 4
        g0 = jnp.pad(h[:, :, 0 * c:1 * c], ((0, 0), (1, 0), (0, 0)))[:, :S, :]
        g1 = jnp.pad(h[:, :, 1 * c:2 * c], ((0, 0), (0, 1), (0, 0)))[:, 1:, :]
        g2 = jnp.pad(h[:, :, 2 * c:3 * c], ((0, 0), (2, 0), (0, 0)))[:, :S, :]
        g3 = jnp.pad(h[:, :, 3 * c:], ((0, 0), (0, 2), (0, 0)))[:, 2:, :]
        hs = jnp.concatenate([g0, g1, g2, g3], axis=-1) @ w2
        x1 = x + hs
        h2 = _gelu(_layernorm(x1, axis=-1) @ w3) @ w4
        return x1 + h2
    x = A_x
    x = x + _A_ref(_layernorm(x, axis=-1), A_wq, A_wk, A_wv, A_wo, A_beta)
    x = x + _B_ref(_layernorm(x, axis=-1), B_w1, B_w2, B_w3, B_w4)
    x = x + _A_ref(_layernorm(x, axis=-1), A_wq, A_wk, A_wv, A_wo, A_beta)
    x = x + _B_ref(_layernorm(x, axis=-1), B_w1, B_w2, B_w3, B_w4)
    return x
```

```python
import functools

import jax
import jax.numpy as jnp
import numpy as np
from jax import lax
import jax.experimental.pallas as pl
import jax.experimental.pallas.tpu as pltpu

S, D, H, DH, NSEG, L, F = 2048, 1024, 32, 32, 4, 512, 3584
G = D // 128
EPS = 1e-5
LOG2E = float(np.log2(np.e))
QSCALE = float(DH ** -0.5) * LOG2E
NEG = -1e9 * LOG2E
GELU_C = float(np.sqrt(2.0 / np.pi))
PAD = 8

F32 = jnp.float32
BF16 = jnp.bfloat16
NT = (((1,), (1,)), ((), ()))


def _ln(x):
    m = jnp.mean(x, axis=-1, keepdims=True)
    d = x - m
    v = jnp.mean(d * d, axis=-1, keepdims=True)
    return d * lax.rsqrt(v + EPS)


def _gelu(x):
    return 0.5 * x * (1.0 + jnp.tanh(GELU_C * (x + 0.044715 * (x * x * x))))


def _phi(t):
    return jnp.where(t > 0, t + 1.0, jnp.exp(t))


def _dot(a, b):
    return jnp.dot(a, b, preferred_element_type=F32)


def _dot_nt(a, b):
    return lax.dot_general(a, b, NT, preferred_element_type=F32)


def _kernel(x_hbm, wq_hbm, wk_hbm, wv_hbm, wo_hbm, beta_ref, w1_hbm, w2_hbm, w3_hbm, w4_hbm,
            out_hbm,
            wq, wk, wv, wo, w1, w2, w3, w4,
            xb, xf, qs, ks, vt, pq, pk, osc, hpad, ysc, gsc, usc, msc, sems, osems):
    TM = 512
    NT_ = S // TM

    cps = [
        pltpu.make_async_copy(x_hbm, xb, sems.at[0]),
        pltpu.make_async_copy(wq_hbm, wq, sems.at[1]),
        pltpu.make_async_copy(wk_hbm, wk, sems.at[2]),
        pltpu.make_async_copy(wv_hbm, wv, sems.at[3]),
        pltpu.make_async_copy(wo_hbm, wo, sems.at[4]),
        pltpu.make_async_copy(w1_hbm, w1, sems.at[5]),
        pltpu.make_async_copy(w2_hbm, w2, sems.at[6]),
        pltpu.make_async_copy(w3_hbm, w3, sems.at[7]),
        pltpu.make_async_copy(w4_hbm, w4, sems.at[8]),
    ]
    for c in cps:
        c.start()

    b = beta_ref[...].astype(F32)
    gv = 1.0 / (1.0 + jnp.exp(-b))
    gb = jnp.broadcast_to(gv, (H, H))
    ri = lax.broadcasted_iota(jnp.int32, (H, H), 0)
    ci = lax.broadcasted_iota(jnp.int32, (H, H), 1)
    gcol = jnp.sum(jnp.where(ri == ci, gb, 0.0), axis=1, keepdims=True)
    gsc[...] = jnp.broadcast_to(gcol, (H, 128))

    for g in range(G):
        hpad[g, pl.ds(0, PAD), :] = jnp.zeros((PAD, 128), F32)
        hpad[g, pl.ds(PAD + S, PAD), :] = jnp.zeros((PAD, 128), F32)

    cps[0].wait()

    def cast_in(i, c):
        r = pl.ds(pl.multiple_of(i * 256, 256), 256)
        xf[r, :] = xb[r, :].astype(F32)
        return c
    lax.fori_loop(0, S // 256, cast_in, 0)

    def stage1(i, c):
        r0 = pl.multiple_of(i * TM, TM)
        rows = pl.ds(r0, TM)
        xn = _ln(xf[rows, :]).astype(BF16)
        for n in range(G // 2):
            cs = slice(n * 256, (n + 1) * 256)
            q = _dot(xn, wq[:, cs])
            qq = (q * QSCALE).astype(BF16)
            ph = _phi(q).astype(BF16)
            for t in range(2):
                qs[2 * n + t, rows, :] = qq[:, t * 128:(t + 1) * 128]
                pq[2 * n + t, rows, :] = ph[:, t * 128:(t + 1) * 128]
        for n in range(G // 2):
            cs = slice(n * 256, (n + 1) * 256)
            k = _dot(xn, wk[:, cs])
            kk = k.astype(BF16)
            ph = _phi(k).astype(BF16)
            for t in range(2):
                ks[2 * n + t, rows, :] = kk[:, t * 128:(t + 1) * 128]
                pk[2 * n + t, rows, :] = ph[:, t * 128:(t + 1) * 128]
        for n in range(G // 2):
            cs = slice(n * 256, (n + 1) * 256)
            v = _dot(xn, wv[:, cs])
            for t in range(2):
                vt[2 * n + t, i, :, :] = jnp.transpose(v[:, t * 128:(t + 1) * 128]).astype(BF16)
        return c

    lane = lax.broadcasted_iota(jnp.int32, (128, 128), 1)
    row = lax.broadcasted_iota(jnp.int32, (128, 128), 0)

    def attn_unit(g, s, first):
        r0 = pl.multiple_of(s * L, L)
        if not first:
            mz = msc[g]
        ocols = []
        for j in range(4):
            qrows = pl.ds(r0 + j * 128, 128)
            qblk = qs[g, qrows, :]
            nk = (j + 1) * 128
            kblk = ks[g, pl.ds(r0, nk), :]
            if not first:
                nd = _dot_nt(mz, pq[g, qrows, :])
            parts = []
            for h in range(4):
                hm = (lane >= h * DH) & (lane < (h + 1) * DH)
                qm = jnp.where(hm, qblk, jnp.zeros_like(qblk))
                st = _dot_nt(kblk, qm)
                diag = st[nk - 128:, :] + jnp.where(row > lane, NEG, 0.0)
                if j > 0:
                    st = jnp.concatenate([st[:nk - 128, :], diag], axis=0)
                else:
                    st = diag
                m = jnp.max(st, axis=0, keepdims=True)
                p = jnp.exp2(st - m)
                l = jnp.sum(p, axis=0, keepdims=True)
                ot = _dot(vt[g, s, pl.ds(h * DH, DH), pl.ds(0, nk)], p.astype(BF16))
                adot = ot / l
                gh = gsc[pl.ds(g * 4 + h, 1), :]
                if first:
                    zero_mem = jnp.zeros((DH, 128), F32) / (jnp.zeros((1, 128), F32) + 1e-6)
                    o = gh * zero_mem + (1.0 - gh) * adot
                else:
                    num = nd[h * DH:(h + 1) * DH, :]
                    den = nd[128 + h:128 + h + 1, :] + 1e-6
                    o = gh * (num / den) + (1.0 - gh) * adot
                parts.append(o)
            ot_all = jnp.concatenate(parts, axis=0)
            osc[g, qrows, :] = jnp.transpose(ot_all).astype(BF16)

    def mem_update(g, s, first):
        r0 = pl.multiple_of(s * L, L)
        pkb = pk[g, pl.ds(r0, L), :]
        mt = _dot(vt[g, s], pkb)
        z = jnp.sum(pkb.astype(F32), axis=0, keepdims=True)
        bd = (row // DH) == (lane // DH)
        mt = jnp.where(bd, mt, 0.0)
        r16 = lax.broadcasted_iota(jnp.int32, (16, 128), 0)
        l16 = lax.broadcasted_iota(jnp.int32, (16, 128), 1)
        zr = jnp.where(r16 == (l16 // DH), jnp.broadcast_to(z, (16, 128)), 0.0)
        upd = jnp.concatenate([mt, zr], axis=0)
        if first:
            acc = upd
        else:
            acc = usc[g] + upd
        usc[g] = acc
        msc[g] = acc.astype(BF16)

    def stage2(c):
        def seg0(g, c):
            attn_unit(g, 0, True)
            mem_update(g, 0, True)
            return c
        lax.fori_loop(0, G, seg0, 0)

        def seg(u, c):
            s = u // G + 1
            g = u % G
            attn_unit(g, s, False)

            @pl.when(s < NSEG - 1)
            def _():
                mem_update(g, s, False)
            return c
        lax.fori_loop(0, G * (NSEG - 1), seg, 0)

    def stage3(i, c):
        r0 = pl.multiple_of(i * TM, TM)
        rows = pl.ds(r0, TM)
        o = jnp.concatenate([osc[g, rows, :] for g in range(G)], axis=1)
        x = xf[rows, :] + _dot(o, wo[...])
        xf[rows, :] = x
        y = _ln(x)
        ysc[rows, :] = y
        yn = _ln(y).astype(BF16)
        for n in range(G // 2):
            hh = _gelu(_dot(yn, w1[:, n * 256:(n + 1) * 256]))
            for t in range(2):
                hpad[2 * n + t, pl.ds(PAD + r0, TM), :] = hh[:, t * 128:(t + 1) * 128]
        return c

    offs = (-1, -1, 1, 1, -2, -2, 2, 2)

    def stage4(i, last):
        r0 = pl.multiple_of(i * TM, TM)
        rows = pl.ds(r0, TM)
        hs_in = jnp.concatenate(
            [hpad[g, pl.ds(PAD + r0 + offs[g], TM), :] for g in range(G)], axis=1).astype(BF16)
        x1 = ysc[rows, :] + _dot(hs_in, w2[...])
        xn = _ln(x1).astype(BF16)
        xf[rows, :] = xf[rows, :] + x1
        for n in range(F // 512):
            cs = slice(n * 512, (n + 1) * 512)
            ub = _gelu(_dot(xn, w3[:, cs])).astype(BF16)
            xf[rows, :] += _dot(ub, w4[cs, :])

        @pl.when(last)
        def _():
            xb[rows, :] = xf[rows, :].astype(BF16)
            pltpu.make_async_copy(xb.at[rows, :], out_hbm.at[rows, :], osems.at[i]).start()

    def layer(it, c):
        @pl.when(it == 0)
        def _():
            cps[1].wait()
            cps[2].wait()
            cps[3].wait()
        lax.fori_loop(0, NT_, stage1, 0)
        stage2(0)

        @pl.when(it == 0)
        def _():
            cps[4].wait()
            cps[5].wait()
        lax.fori_loop(0, NT_, stage3, 0)

        @pl.when(it == 0)
        def _():
            cps[6].wait()
            cps[7].wait()
            cps[8].wait()

        def s4(i, c):
            stage4(i, it == 1)
            return c
        lax.fori_loop(0, NT_, s4, 0)
        return c

    lax.fori_loop(0, 2, layer, 0)

    for i in range(NT_):
        rows = pl.ds(i * TM, TM)
        pltpu.make_async_copy(xb.at[rows, :], out_hbm.at[rows, :], osems.at[i]).wait()


@jax.jit
def pallas_interleave_layers__memory_aug_infini_attn__mixer_s_mlp__prompt_kernel(
    A_x: jax.Array,
    A_wq: jax.Array,
    A_wk: jax.Array,
    A_wv: jax.Array,
    A_wo: jax.Array,
    A_beta: jax.Array,
    B_x: jax.Array,
    B_w1: jax.Array,
    B_w2: jax.Array,
    B_w3: jax.Array,
    B_w4: jax.Array,
):
    del B_x
    x = A_x.reshape(S, D)
    beta = A_beta.reshape(1, H)
    any_spec = pl.BlockSpec(memory_space=pl.ANY)
    scratch = [
        pltpu.VMEM((D, D), BF16), pltpu.VMEM((D, D), BF16), pltpu.VMEM((D, D), BF16),
        pltpu.VMEM((D, D), BF16), pltpu.VMEM((D, D), BF16), pltpu.VMEM((D, D), BF16),
        pltpu.VMEM((D, F), BF16), pltpu.VMEM((F, D), BF16),
        pltpu.VMEM((S, D), BF16),
        pltpu.VMEM((S, D), F32),
        pltpu.VMEM((G, S, 128), BF16),
        pltpu.VMEM((G, S, 128), BF16),
        pltpu.VMEM((G, NSEG, 128, L), BF16),
        pltpu.VMEM((G, S, 128), BF16),
        pltpu.VMEM((G, S, 128), BF16),
        pltpu.VMEM((G, S, 128), BF16),
        pltpu.VMEM((G, S + 2 * PAD, 128), F32),
        pltpu.VMEM((S, D), F32),
        pltpu.VMEM((H, 128), F32),
        pltpu.VMEM((G, 144, 128), F32),
        pltpu.VMEM((G, 144, 128), BF16),
        pltpu.SemaphoreType.DMA((9,)),
        pltpu.SemaphoreType.DMA((4,)),
    ]
    out = pl.pallas_call(
        _kernel,
        out_shape=jax.ShapeDtypeStruct((S, D), BF16),
        in_specs=[any_spec] * 5 + [pl.BlockSpec(memory_space=pltpu.VMEM)] + [any_spec] * 4,
        out_specs=any_spec,
        scratch_shapes=scratch,
        compiler_params=pltpu.CompilerParams(vmem_limit_bytes=120 * 1024 * 1024),
    )(x, A_wq, A_wk, A_wv, A_wo, beta, B_w1, B_w2, B_w3, B_w4)
    return out.reshape(1, S, D)
```

```python
import functools

import jax
import jax.numpy as jnp
import numpy as np
from jax import lax
import jax.experimental.pallas as pl
import jax.experimental.pallas.tpu as pltpu

S, D, H, DH, NSEG, L, F = 2048, 1024, 32, 32, 4, 512, 3584
G = D // 128
EPS = 1e-5
LOG2E = float(np.log2(np.e))
QSCALE = float(DH ** -0.5) * LOG2E
NEG = -1e9 * LOG2E
GELU_C = float(np.sqrt(2.0 / np.pi))
PAD = 8
OFF = (0, 128, 384, 768)
TILES = tuple((j, kb) for j in range(4) for kb in range(j + 1))

F32 = jnp.float32
BF16 = jnp.bfloat16
NT = (((1,), (1,)), ((), ()))


def _ln(x):
    m = jnp.mean(x, axis=-1, keepdims=True)
    d = x - m
    v = jnp.mean(d * d, axis=-1, keepdims=True)
    return d * lax.rsqrt(v + EPS)


def _gelu(x):
    return 0.5 * x * (1.0 + jnp.tanh(GELU_C * (x + 0.044715 * (x * x * x))))


def _phi(t):
    return jnp.where(t > 0, t + 1.0, jnp.exp(t))


def _dot(a, b):
    return jnp.dot(a, b, preferred_element_type=F32)


def _dot_nt(a, b):
    return lax.dot_general(a, b, NT, preferred_element_type=F32)


def _kernel(x_hbm, wq_hbm, wk_hbm, wv_hbm, wo_hbm, beta_ref, w1_hbm, w2_hbm, w3_hbm, w4_hbm,
            out_hbm,
            wq, wk, wv, wo, w1, w2, w3, w4,
            xb, xf, qs, ks, vt, pq, pk, osc, hpad, ysc, gsc, usc, msc,
            s_a, s_b, m_a, m_b, p_a, p_b, l_a, l_b, t_a, t_b, bsc, sems, osems):
    TM = 512
    NT_ = S // TM

    cps = [
        pltpu.make_async_copy(x_hbm, xb, sems.at[0]),
        pltpu.make_async_copy(wq_hbm, wq, sems.at[1]),
        pltpu.make_async_copy(wk_hbm, wk, sems.at[2]),
        pltpu.make_async_copy(wv_hbm, wv, sems.at[3]),
        pltpu.make_async_copy(wo_hbm, wo, sems.at[4]),
        pltpu.make_async_copy(w1_hbm, w1, sems.at[5]),
        pltpu.make_async_copy(w2_hbm, w2, sems.at[6]),
        pltpu.make_async_copy(w3_hbm, w3, sems.at[7]),
        pltpu.make_async_copy(w4_hbm, w4, sems.at[8]),
    ]
    for c in cps:
        c.start()

    b = beta_ref[...].astype(F32)
    gv = 1.0 / (1.0 + jnp.exp(-b))
    gb = jnp.broadcast_to(gv, (H, H))
    ri = lax.broadcasted_iota(jnp.int32, (H, H), 0)
    ci = lax.broadcasted_iota(jnp.int32, (H, H), 1)
    gcol = jnp.sum(jnp.where(ri == ci, gb, 0.0), axis=1, keepdims=True)
    gsc[...] = jnp.broadcast_to(gcol, (H, 128))

    for g in range(G):
        hpad[g, pl.ds(0, PAD), :] = jnp.zeros((PAD, 128), F32)
        hpad[g, pl.ds(PAD + S, PAD), :] = jnp.zeros((PAD, 128), F32)

    cps[0].wait()

    def cast_in(i, c):
        r = pl.ds(pl.multiple_of(i * 256, 256), 256)
        xf[r, :] = xb[r, :].astype(F32)
        return c
    lax.fori_loop(0, S // 256, cast_in, 0)

    def stage1(i, c):
        r0 = pl.multiple_of(i * TM, TM)
        rows = pl.ds(r0, TM)
        xn = _ln(xf[rows, :]).astype(BF16)
        for n in range(G // 2):
            cs = slice(n * 256, (n + 1) * 256)
            q = _dot(xn, wq[:, cs])
            qq = (q * QSCALE).astype(BF16)
            ph = _phi(q).astype(BF16)
            for t in range(2):
                qs[2 * n + t, rows, :] = qq[:, t * 128:(t + 1) * 128]
                pq[2 * n + t, rows, :] = ph[:, t * 128:(t + 1) * 128]
        for n in range(G // 2):
            cs = slice(n * 256, (n + 1) * 256)
            k = _dot(xn, wk[:, cs])
            kk = k.astype(BF16)
            ph = _phi(k).astype(BF16)
            for t in range(2):
                ks[2 * n + t, rows, :] = kk[:, t * 128:(t + 1) * 128]
                pk[2 * n + t, rows, :] = ph[:, t * 128:(t + 1) * 128]
        for n in range(G // 2):
            cs = slice(n * 256, (n + 1) * 256)
            v = _dot(xn, wv[:, cs])
            for t in range(2):
                vt[2 * n + t, i, :, :] = jnp.transpose(v[:, t * 128:(t + 1) * 128]).astype(BF16)
        return c

    lane = lax.broadcasted_iota(jnp.int32, (128, 128), 1)
    row = lax.broadcasted_iota(jnp.int32, (128, 128), 0)
    bsc[...] = jnp.where(row > lane, NEG, 0.0)
    NU = G * NSEG

    def step_qk(u, j, kb, s_scr, m_scr, st):
        s = u // G
        g = u % G
        r0 = pl.multiple_of(s * L, L)
        if kb == 0:
            lane64 = lax.broadcasted_iota(jnp.int32, (64, 128), 1)
            qi = pltpu.bitcast(qs[g, pl.ds(r0 + j * 128, 128), :], jnp.int32)
            st["q"] = jnp.concatenate(
                [pltpu.bitcast(jnp.where((lane64 // DH) == h, qi, 0), BF16) for h in range(4)], axis=0)
            st["mx"] = [None] * 4
        sq = _dot_nt(ks[g, pl.ds(r0 + kb * 128, 128), :], st["q"])
        o = OFF[j] + kb * 128
        for h in range(4):
            t = sq[:, h * 128:(h + 1) * 128]
            if kb == j:
                t = t + bsc[...]
            s_scr[h, o:o + 128, :] = t
            tm = jnp.max(t.reshape(16, 8, 128), axis=0)
            st["mx"][h] = tm if kb == 0 else jnp.maximum(st["mx"][h], tm)
            if kb == j:
                m_scr[j, h] = jnp.broadcast_to(jnp.max(st["mx"][h], axis=0, keepdims=True), (8, 128))

    def step_ex(j, kb, s_scr, m_scr, p_scr, l_scr, st):
        o = OFF[j] + kb * 128
        if kb == 0:
            st["ls"] = [None] * 4
        for h in range(4):
            t = s_scr[h, o:o + 128, :]
            p = jnp.exp2(t.reshape(16, 8, 128) - m_scr[j, h][None])
            ps = jnp.sum(p, axis=0)
            st["ls"][h] = ps if kb == 0 else st["ls"][h] + ps
            p_scr[h, o:o + 128, :] = p.reshape(128, 128).astype(BF16)
            if kb == j:
                l_scr[j, h] = jnp.broadcast_to(jnp.sum(st["ls"][h], axis=0, keepdims=True), (8, 128))

    def step_pv(u, j, kb, p_scr, l_scr, t_scr, st):
        s = u // G
        g = u % G
        r0 = pl.multiple_of(s * L, L)
        o = OFF[j] + kb * 128
        if kb == 0:
            st["acc"] = [None] * 4
        for h in range(4):
            r = _dot(vt[g, s, pl.ds(h * DH, DH), pl.ds(kb * 128, 128)], p_scr[h, o:o + 128, :])
            st["acc"][h] = r if kb == 0 else st["acc"][h] + r
        if kb == j:
            nd = _dot_nt(msc[g], pq[g, pl.ds(r0 + j * 128, 128), :])
            for h in range(4):
                gh = jnp.broadcast_to(gsc[pl.ds(g * 4 + h, 1), :], (8, 128))
                den = jnp.broadcast_to(nd[128 + h:128 + h + 1, :], (8, 128)) + 1e-6
                cm = gh / den
                cd = (1.0 - gh) / l_scr[j, h]
                num = nd[h * DH:(h + 1) * DH, :].reshape(4, 8, 128)
                acc = st["acc"][h].reshape(4, 8, 128)
                t_scr[h * DH:(h + 1) * DH, j * 128:(j + 1) * 128] = (num * cm[None] + acc * cd[None]).reshape(DH, 128)

    def mem_update(u):
        s = u // G
        g = u % G
        r0 = pl.multiple_of(s * L, L)
        lhs = jnp.concatenate([vt[g, s], jnp.ones((16, L), BF16)], axis=0)
        upd = _dot(lhs, pk[g, pl.ds(r0, L), :])
        r144 = lax.broadcasted_iota(jnp.int32, (144, 128), 0)
        l144 = lax.broadcasted_iota(jnp.int32, (144, 128), 1)
        rh = jnp.where(r144 < 128, r144 // DH, r144 - 128)
        acc = usc[g] + jnp.where(rh == l144 // DH, upd, 0.0)
        usc[g] = acc
        msc[g] = acc.astype(BF16)

    def step_t(u, t_scr):
        s = u // G
        g = u % G
        r0 = pl.multiple_of(s * L, L)
        for j in range(4):
            osc[g, pl.ds(r0 + j * 128, 128), :] = jnp.transpose(t_scr[:, j * 128:(j + 1) * 128]).astype(BF16)

    def fused(u, cur, nxt):
        a, b, c = {}, {}, {}
        un = jnp.minimum(u + 2, NU - 1)
        step_t(jnp.maximum(u - 1, 0), nxt[4])
        for (j, kb) in TILES:
            step_pv(u, j, kb, cur[2], cur[3], cur[4], a)
            step_ex(j, kb, nxt[0], nxt[1], nxt[2], nxt[3], b)
            step_qk(un, j, kb, cur[0], cur[1], c)
        mem_update(u)

    def stage2(c):
        set_a = (s_a, m_a, p_a, l_a, t_a)
        set_b = (s_b, m_b, p_b, l_b, t_b)
        usc[...] = jnp.zeros(usc.shape, F32)
        msc[...] = jnp.zeros(msc.shape, BF16)
        t_b[...] = jnp.zeros(t_b.shape, F32)
        st = {}
        for (j, kb) in TILES:
            step_qk(0, j, kb, s_a, m_a, st)
        for (j, kb) in TILES:
            step_qk(1, j, kb, s_b, m_b, st)
            step_ex(j, kb, s_a, m_a, p_a, l_a, st)

        def one(u, c):
            @pl.when(u % 2 == 0)
            def _():
                fused(u, set_a, set_b)

            @pl.when(u % 2 == 1)
            def _():
                fused(u, set_b, set_a)
            return c
        lax.fori_loop(0, NU, one, 0)
        step_t(NU - 1, t_b)

    def stage3(i, c):
        r0 = pl.multiple_of(i * TM, TM)
        rows = pl.ds(r0, TM)
        o = jnp.concatenate([osc[g, rows, :] for g in range(G)], axis=1)
        x = xf[rows, :] + _dot(o, wo[...])
        xf[rows, :] = x
        y = _ln(x)
        ysc[rows, :] = y
        yn = _ln(y).astype(BF16)
        for n in range(G // 2):
            hh = _gelu(_dot(yn, w1[:, n * 256:(n + 1) * 256]))
            for t in range(2):
                hpad[2 * n + t, pl.ds(PAD + r0, TM), :] = hh[:, t * 128:(t + 1) * 128]
        return c

    offs = (-1, -1, 1, 1, -2, -2, 2, 2)

    def stage4(i, last):
        r0 = pl.multiple_of(i * TM, TM)
        rows = pl.ds(r0, TM)
        hs_in = jnp.concatenate(
            [hpad[g, pl.ds(PAD + r0 + offs[g], TM), :] for g in range(G)], axis=1).astype(BF16)
        x1 = ysc[rows, :] + _dot(hs_in, w2[...])
        xn = _ln(x1).astype(BF16)
        xf[rows, :] = xf[rows, :] + x1
        for n in range(F // 512):
            cs = slice(n * 512, (n + 1) * 512)
            ub = _gelu(_dot(xn, w3[:, cs])).astype(BF16)
            xf[rows, :] += _dot(ub, w4[cs, :])

        @pl.when(last)
        def _():
            xb[rows, :] = xf[rows, :].astype(BF16)
            pltpu.make_async_copy(xb.at[rows, :], out_hbm.at[rows, :], osems.at[i]).start()

    def layer(it, c):
        @pl.when(it == 0)
        def _():
            cps[1].wait()
            cps[2].wait()
            cps[3].wait()
        lax.fori_loop(0, NT_, stage1, 0)
        stage2(0)

        @pl.when(it == 0)
        def _():
            cps[4].wait()
            cps[5].wait()
        lax.fori_loop(0, NT_, stage3, 0)

        @pl.when(it == 0)
        def _():
            cps[6].wait()
            cps[7].wait()
            cps[8].wait()

        def s4(i, c):
            stage4(i, it == 1)
            return c
        lax.fori_loop(0, NT_, s4, 0)
        return c

    lax.fori_loop(0, 2, layer, 0)

    for i in range(NT_):
        rows = pl.ds(i * TM, TM)
        pltpu.make_async_copy(xb.at[rows, :], out_hbm.at[rows, :], osems.at[i]).wait()


@jax.jit
def pallas_interleave_layers__memory_aug_infini_attn__mixer_s_mlp__prompt_kernel(
    A_x: jax.Array,
    A_wq: jax.Array,
    A_wk: jax.Array,
    A_wv: jax.Array,
    A_wo: jax.Array,
    A_beta: jax.Array,
    B_x: jax.Array,
    B_w1: jax.Array,
    B_w2: jax.Array,
    B_w3: jax.Array,
    B_w4: jax.Array,
):
    del B_x
    x = A_x.reshape(S, D)
    beta = A_beta.reshape(1, H)
    any_spec = pl.BlockSpec(memory_space=pl.ANY)
    scratch = [
        pltpu.VMEM((D, D), BF16), pltpu.VMEM((D, D), BF16), pltpu.VMEM((D, D), BF16),
        pltpu.VMEM((D, D), BF16), pltpu.VMEM((D, D), BF16), pltpu.VMEM((D, D), BF16),
        pltpu.VMEM((D, F), BF16), pltpu.VMEM((F, D), BF16),
        pltpu.VMEM((S, D), BF16),
        pltpu.VMEM((S, D), F32),
        pltpu.VMEM((G, S, 128), BF16),
        pltpu.VMEM((G, S, 128), BF16),
        pltpu.VMEM((G, NSEG, 128, L), BF16),
        pltpu.VMEM((G, S, 128), BF16),
        pltpu.VMEM((G, S, 128), BF16),
        pltpu.VMEM((G, S, 128), BF16),
        pltpu.VMEM((G, S + 2 * PAD, 128), F32),
        pltpu.VMEM((S, D), F32),
        pltpu.VMEM((H, 128), F32),
        pltpu.VMEM((G, 144, 128), F32),
        pltpu.VMEM((G, 144, 128), BF16),
        pltpu.VMEM((4, 1280, 128), F32), pltpu.VMEM((4, 1280, 128), F32),
        pltpu.VMEM((4, 4, 8, 128), F32), pltpu.VMEM((4, 4, 8, 128), F32),
        pltpu.VMEM((4, 1280, 128), BF16), pltpu.VMEM((4, 1280, 128), BF16),
        pltpu.VMEM((4, 4, 8, 128), F32), pltpu.VMEM((4, 4, 8, 128), F32),
        pltpu.VMEM((128, L), F32), pltpu.VMEM((128, L), F32),
        pltpu.VMEM((128, 128), F32),
        pltpu.SemaphoreType.DMA((9,)),
        pltpu.SemaphoreType.DMA((4,)),
    ]
    out = pl.pallas_call(
        _kernel,
        out_shape=jax.ShapeDtypeStruct((S, D), BF16),
        in_specs=[any_spec] * 5 + [pl.BlockSpec(memory_space=pltpu.VMEM)] + [any_spec] * 4,
        out_specs=any_spec,
        scratch_shapes=scratch,
        compiler_params=pltpu.CompilerParams(vmem_limit_bytes=120 * 1024 * 1024),
    )(x, A_wq, A_wk, A_wv, A_wo, beta, B_w1, B_w2, B_w3, B_w4)
    return out.reshape(1, S, D)
```

```python
import contextlib
import functools

import jax
import jax.numpy as jnp
import numpy as np
from jax import lax
import jax.experimental.pallas as pl
import jax.experimental.pallas.tpu as pltpu

S, D, H, DH, NSEG, L, F = 2048, 1024, 32, 32, 4, 512, 3584
G = D // 128
EPS = 1e-5
LOG2E = float(np.log2(np.e))
QSCALE = float(DH ** -0.5) * LOG2E
NEG = -1e9 * LOG2E
GELU_C = float(np.sqrt(2.0 / np.pi))
PAD = 8
MC = 128
FC = 512
NFC = F // FC
OFF = (0, 128, 384, 768)
TILES = tuple((j, kb) for j in range(4) for kb in range(j + 1))

PROFILE = False


def _scope(name):
    return jax.named_scope(name) if PROFILE else contextlib.nullcontext()


F32 = jnp.float32
BF16 = jnp.bfloat16
NT = (((1,), (1,)), ((), ()))


def _ln(x):
    m = jnp.mean(x, axis=-1, keepdims=True)
    d = x - m
    v = jnp.mean(d * d, axis=-1, keepdims=True)
    return d * lax.rsqrt(v + EPS)


def _gelu(x):
    return 0.5 * x * (1.0 + jnp.tanh(GELU_C * (x + 0.044715 * (x * x * x))))


def _phi(t):
    return jnp.where(t > 0, t + 1.0, jnp.exp(t))


def _dot(a, b):
    return jnp.dot(a, b, preferred_element_type=F32)


def _dot_nt(a, b):
    return lax.dot_general(a, b, NT, preferred_element_type=F32)


def _kernel(x_hbm, wq_hbm, wk_hbm, wv_hbm, wo_hbm, beta_ref, w1_hbm, w2_hbm, w3_hbm, w4_hbm,
            out_hbm,
            wq, wk, wv, wo, w1, w2, w3, w4,
            xb, xf, qs, ks, vt, pq, pk, osc, hpad, ysc, gsc, usc, msc,
            s_a, s_b, m_a, m_b, p_a, p_b, l_a, l_b, t_a, t_b, bsc, xa, xc, sems, osems, w3sems, xsems):
    TM = 512
    NT_ = S // TM

    xcps = [pltpu.make_async_copy(x_hbm.at[pl.ds(i * TM, TM), :], xb.at[pl.ds(i * TM, TM), :], xsems.at[i])
            for i in range(NT_)]
    wcps = [
        pltpu.make_async_copy(wq_hbm, wq, sems.at[0]),
        pltpu.make_async_copy(wk_hbm, wk, sems.at[1]),
        pltpu.make_async_copy(wv_hbm, wv, sems.at[2]),
        pltpu.make_async_copy(wo_hbm, wo, sems.at[3]),
        pltpu.make_async_copy(w1_hbm, w1, sems.at[4]),
        pltpu.make_async_copy(w2_hbm, w2, sems.at[5]),
        pltpu.make_async_copy(w4_hbm, w4, sems.at[6]),
    ]
    w3cps = [pltpu.make_async_copy(w3_hbm.at[:, pl.ds(n * FC, FC)], w3.at[n], w3sems.at[n]) for n in range(NFC)]
    xcps[0].start()
    wcps[0].start()
    xcps[1].start()

    b = beta_ref[...].astype(F32)
    gv = 1.0 / (1.0 + jnp.exp(-b))
    gb = jnp.broadcast_to(gv, (H, H))
    ri = lax.broadcasted_iota(jnp.int32, (H, H), 0)
    ci = lax.broadcasted_iota(jnp.int32, (H, H), 1)
    gcol = jnp.sum(jnp.where(ri == ci, gb, 0.0), axis=1, keepdims=True)
    gsc[...] = jnp.broadcast_to(gcol, (H, 128))

    for g in range(G):
        hpad[g, pl.ds(0, PAD), :] = jnp.zeros((PAD, 128), F32)
        hpad[g, pl.ds(PAD + S, PAD), :] = jnp.zeros((PAD, 128), F32)

    def trows(i, n=TM):
        return pl.ds(pl.multiple_of(i * TM, TM), n)

    def xcur(rows, first):
        return jnp.where(first, xb[rows, :].astype(F32), xf[rows, :])

    def stage1(first):
        @pl.when(first)
        def _():
            with _scope("xwait"):
                xcps[0].wait()
                wcps[0].wait()
            for c_ in (xcps[2], xcps[3], wcps[1]):
                c_.start()

        def qloop(i, c):
            @pl.when(first & (i >= 1))
            def _():
                pltpu.make_async_copy(x_hbm.at[trows(i), :], xb.at[trows(i), :], xsems.at[i]).wait()
            for mc in range(TM // MC):
                rows = pl.ds(pl.multiple_of(i * TM + mc * MC, MC), MC)
                x = _ln(xcur(rows, first)).astype(BF16)
                xa[rows, :] = x
                q = _dot(x, wq[...])
                qq = (q * QSCALE).astype(BF16)
                ph = _phi(q).astype(BF16)
                for t in range(G):
                    qs[t, rows, :] = qq[:, t * 128:(t + 1) * 128]
                    pq[t, rows, :] = ph[:, t * 128:(t + 1) * 128]
            return c
        lax.fori_loop(0, NT_, qloop, 0)

        @pl.when(first)
        def _():
            for c_ in (wcps[2], wcps[3], wcps[4]):
                c_.start()
            wcps[1].wait()

        def kloop(i, c):
            rows = trows(i)
            x = xa[trows(i), :]
            for n in range(G // 2):
                k = _dot(x, wk[:, n * 256:(n + 1) * 256])
                kk = k.astype(BF16)
                ph = _phi(k).astype(BF16)
                for t in range(2):
                    ks[2 * n + t, rows, :] = kk[:, t * 128:(t + 1) * 128]
                    pk[2 * n + t, rows, :] = ph[:, t * 128:(t + 1) * 128]
            return c
        lax.fori_loop(0, NT_, kloop, 0)

        @pl.when(first)
        def _():
            for c_ in (wcps[5],) + tuple(w3cps) + (wcps[6],):
                c_.start()
            wcps[2].wait()

        def vloop(i, c):
            x = xa[trows(i), :]
            for n in range(G // 2):
                v = _dot(x, wv[:, n * 256:(n + 1) * 256])
                for t in range(2):
                    vt[2 * n + t, i, :, :] = jnp.transpose(v[:, t * 128:(t + 1) * 128]).astype(BF16)
            return c
        lax.fori_loop(0, NT_, vloop, 0)

    lane = lax.broadcasted_iota(jnp.int32, (128, 128), 1)
    row = lax.broadcasted_iota(jnp.int32, (128, 128), 0)
    bsc[...] = jnp.where(row > lane, NEG, 0.0)
    NU = G * NSEG

    def step_qk(u, j, kb, s_scr, m_scr, st):
        s = u // G
        g = u % G
        r0 = pl.multiple_of(s * L, L)
        if kb == 0:
            lane64 = lax.broadcasted_iota(jnp.int32, (64, 128), 1)
            qi = pltpu.bitcast(qs[g, pl.ds(r0 + j * 128, 128), :], jnp.int32)
            st["q"] = jnp.concatenate(
                [pltpu.bitcast(jnp.where((lane64 // DH) == h, qi, 0), BF16) for h in range(4)], axis=0)
            st["mx"] = [None] * 4
        sq = _dot_nt(ks[g, pl.ds(r0 + kb * 128, 128), :], st["q"])
        o = OFF[j] + kb * 128
        for h in range(4):
            t = sq[:, h * 128:(h + 1) * 128]
            if kb == j:
                t = t + bsc[...]
            s_scr[h, o:o + 128, :] = t
            tm = jnp.max(t.reshape(16, 8, 128), axis=0)
            st["mx"][h] = tm if kb == 0 else jnp.maximum(st["mx"][h], tm)
            if kb == j:
                m_scr[j, h] = jnp.broadcast_to(jnp.max(st["mx"][h], axis=0, keepdims=True), (8, 128))

    def step_ex(j, kb, s_scr, m_scr, p_scr, l_scr, st):
        o = OFF[j] + kb * 128
        if kb == 0:
            st["ls"] = [None] * 4
        for h in range(4):
            t = s_scr[h, o:o + 128, :]
            p = jnp.exp2(t.reshape(16, 8, 128) - m_scr[j, h][None])
            ps = jnp.sum(p, axis=0)
            st["ls"][h] = ps if kb == 0 else st["ls"][h] + ps
            p_scr[h, o:o + 128, :] = p.reshape(128, 128).astype(BF16)
            if kb == j:
                l_scr[j, h] = jnp.broadcast_to(jnp.sum(st["ls"][h], axis=0, keepdims=True), (8, 128))

    def step_pv(u, j, kb, p_scr, l_scr, t_scr, st):
        s = u // G
        g = u % G
        r0 = pl.multiple_of(s * L, L)
        o = OFF[j] + kb * 128
        if kb == 0:
            st["acc"] = [None] * 4
        for h in range(4):
            r = _dot(vt[g, s, pl.ds(h * DH, DH), pl.ds(kb * 128, 128)], p_scr[h, o:o + 128, :])
            st["acc"][h] = r if kb == 0 else st["acc"][h] + r
        if kb == j:
            nd = _dot_nt(msc[g], pq[g, pl.ds(r0 + j * 128, 128), :])
            for h in range(4):
                gh = jnp.broadcast_to(gsc[pl.ds(g * 4 + h, 1), :], (8, 128))
                den = jnp.broadcast_to(nd[128 + h:128 + h + 1, :], (8, 128)) + 1e-6
                cm = gh / den
                cd = (1.0 - gh) / l_scr[j, h]
                num = nd[h * DH:(h + 1) * DH, :].reshape(4, 8, 128)
                acc = st["acc"][h].reshape(4, 8, 128)
                t_scr[h * DH:(h + 1) * DH, j * 128:(j + 1) * 128] = (num * cm[None] + acc * cd[None]).reshape(DH, 128)

    def mem_update(u):
        s = u // G
        g = u % G
        r0 = pl.multiple_of(s * L, L)
        lhs = jnp.concatenate([vt[g, s], jnp.ones((16, L), BF16)], axis=0)
        upd = _dot(lhs, pk[g, pl.ds(r0, L), :])
        r144 = lax.broadcasted_iota(jnp.int32, (144, 128), 0)
        l144 = lax.broadcasted_iota(jnp.int32, (144, 128), 1)
        rh = jnp.where(r144 < 128, r144 // DH, r144 - 128)
        acc = usc[g] + jnp.where(rh == l144 // DH, upd, 0.0)
        usc[g] = acc
        msc[g] = acc.astype(BF16)

    def step_t(u, t_scr):
        s = u // G
        g = u % G
        r0 = pl.multiple_of(s * L, L)
        for j in range(4):
            osc[g, pl.ds(r0 + j * 128, 128), :] = jnp.transpose(t_scr[:, j * 128:(j + 1) * 128]).astype(BF16)

    def fused(u, cur, nxt):
        a, b, c = {}, {}, {}
        un = jnp.minimum(u + 2, NU - 1)
        step_t(jnp.maximum(u - 1, 0), nxt[4])
        for (j, kb) in TILES:
            step_pv(u, j, kb, cur[2], cur[3], cur[4], a)
            step_ex(j, kb, nxt[0], nxt[1], nxt[2], nxt[3], b)
            step_qk(un, j, kb, cur[0], cur[1], c)
        mem_update(u)

    def stage2(c):
        set_a = (s_a, m_a, p_a, l_a, t_a)
        set_b = (s_b, m_b, p_b, l_b, t_b)
        usc[...] = jnp.zeros(usc.shape, F32)
        msc[...] = jnp.zeros(msc.shape, BF16)
        t_b[...] = jnp.zeros(t_b.shape, F32)
        st = {}
        for (j, kb) in TILES:
            step_qk(0, j, kb, s_a, m_a, st)
        for (j, kb) in TILES:
            step_qk(1, j, kb, s_b, m_b, st)
            step_ex(j, kb, s_a, m_a, p_a, l_a, st)

        def one(u, c):
            @pl.when(u % 2 == 0)
            def _():
                fused(u, set_a, set_b)

            @pl.when(u % 2 == 1)
            def _():
                fused(u, set_b, set_a)
            return c
        lax.fori_loop(0, NU, one, 0)
        step_t(NU - 1, t_b)

    def stage3(first):
        def body(i, c):
            yns = []
            for mc in range(TM // MC):
                rows = pl.ds(pl.multiple_of(i * TM + mc * MC, MC), MC)
                o = jnp.concatenate([osc[g, rows, :] for g in range(G)], axis=1)
                x = xcur(rows, first) + _dot(o, wo[...])
                xf[rows, :] = x
                y = _ln(x)
                ysc[rows, :] = y
                yns.append(_ln(y).astype(BF16))
            for mc in range(TM // MC):
                r0 = pl.multiple_of(i * TM + mc * MC, MC)
                hh = _gelu(_dot(yns[mc], w1[...]))
                for t in range(G):
                    hpad[t, pl.ds(PAD + r0, MC), :] = hh[:, t * 128:(t + 1) * 128]
            return c
        lax.fori_loop(0, NT_, body, 0)

    offs = (-1, -1, 1, 1, -2, -2, 2, 2)

    def stage4(last):
        def body(i, c):
            for mc in range(TM // MC):
                r0 = pl.multiple_of(i * TM + mc * MC, MC)
                rows = pl.ds(r0, MC)
                hs_in = jnp.concatenate(
                    [hpad[g, pl.ds(PAD + r0 + offs[g], MC), :] for g in range(G)], axis=1).astype(BF16)
                x1 = ysc[rows, :] + _dot(hs_in, w2[...])
                xf[rows, :] = xf[rows, :] + x1
                xc[mc * MC:(mc + 1) * MC, :] = _ln(x1).astype(BF16)
            rows = trows(i)

            def ffn(n, c):
                ub = _gelu(_dot(xc[...], w3[n])).astype(BF16)
                xf[rows, :] += _dot(ub, w4[n])
                return c
            lax.fori_loop(0, NFC, ffn, 0)

            @pl.when(last)
            def _():
                xb[rows, :] = xf[rows, :].astype(BF16)
                pltpu.make_async_copy(xb.at[rows, :], out_hbm.at[rows, :], osems.at[i]).start()
            return c
        lax.fori_loop(0, NT_, body, 0)

    def layer(it, c):
        first = it == 0
        with _scope("stage1"):
            stage1(first)
        with _scope("stage2"):
            stage2(0)

        @pl.when(first)
        def _():
            wcps[3].wait()
            wcps[4].wait()
        with _scope("stage3"):
            stage3(first)

        @pl.when(first)
        def _():
            wcps[5].wait()
            for c_ in w3cps:
                c_.wait()
            wcps[6].wait()
        with _scope("stage4"):
            stage4(it == 1)
        return c

    lax.fori_loop(0, 2, layer, 0)

    for i in range(NT_):
        rows = pl.ds(i * TM, TM)
        pltpu.make_async_copy(xb.at[rows, :], out_hbm.at[rows, :], osems.at[i]).wait()


@jax.jit
def pallas_interleave_layers__memory_aug_infini_attn__mixer_s_mlp__prompt_kernel(
    A_x: jax.Array,
    A_wq: jax.Array,
    A_wk: jax.Array,
    A_wv: jax.Array,
    A_wo: jax.Array,
    A_beta: jax.Array,
    B_x: jax.Array,
    B_w1: jax.Array,
    B_w2: jax.Array,
    B_w3: jax.Array,
    B_w4: jax.Array,
):
    del B_x
    x = A_x.reshape(S, D)
    beta = A_beta.reshape(1, H)
    any_spec = pl.BlockSpec(memory_space=pl.ANY)
    scratch = [
        pltpu.VMEM((D, D), BF16), pltpu.VMEM((D, D), BF16), pltpu.VMEM((D, D), BF16),
        pltpu.VMEM((D, D), BF16), pltpu.VMEM((D, D), BF16), pltpu.VMEM((D, D), BF16),
        pltpu.VMEM((NFC, D, FC), BF16), pltpu.VMEM((NFC, FC, D), BF16),
        pltpu.VMEM((S, D), BF16),
        pltpu.VMEM((S, D), F32),
        pltpu.VMEM((G, S, 128), BF16),
        pltpu.VMEM((G, S, 128), BF16),
        pltpu.VMEM((G, NSEG, 128, L), BF16),
        pltpu.VMEM((G, S, 128), BF16),
        pltpu.VMEM((G, S, 128), BF16),
        pltpu.VMEM((G, S, 128), BF16),
        pltpu.VMEM((G, S + 2 * PAD, 128), F32),
        pltpu.VMEM((S, D), F32),
        pltpu.VMEM((H, 128), F32),
        pltpu.VMEM((G, 144, 128), F32),
        pltpu.VMEM((G, 144, 128), BF16),
        pltpu.VMEM((4, 1280, 128), F32), pltpu.VMEM((4, 1280, 128), F32),
        pltpu.VMEM((4, 4, 8, 128), F32), pltpu.VMEM((4, 4, 8, 128), F32),
        pltpu.VMEM((4, 1280, 128), BF16), pltpu.VMEM((4, 1280, 128), BF16),
        pltpu.VMEM((4, 4, 8, 128), F32), pltpu.VMEM((4, 4, 8, 128), F32),
        pltpu.VMEM((128, L), F32), pltpu.VMEM((128, L), F32),
        pltpu.VMEM((128, 128), F32),
        pltpu.VMEM((S, D), BF16), pltpu.VMEM((512, D), BF16),
        pltpu.SemaphoreType.DMA((7,)),
        pltpu.SemaphoreType.DMA((4,)),
        pltpu.SemaphoreType.DMA((NFC,)),
        pltpu.SemaphoreType.DMA((4,)),
    ]
    out = pl.pallas_call(
        _kernel,
        out_shape=jax.ShapeDtypeStruct((S, D), BF16),
        in_specs=[any_spec] * 5 + [pl.BlockSpec(memory_space=pltpu.VMEM)] + [any_spec] * 4,
        out_specs=any_spec,
        scratch_shapes=scratch,
        compiler_params=pltpu.CompilerParams(vmem_limit_bytes=120 * 1024 * 1024),
    )(x, A_wq, A_wk, A_wv, A_wo, beta, B_w1, B_w2, B_w3, B_w4.reshape(NFC, FC, D))
    return out.reshape(1, S, D)
```

```python
import contextlib
import functools

import jax
import jax.numpy as jnp
import numpy as np
from jax import lax
import jax.experimental.pallas as pl
import jax.experimental.pallas.tpu as pltpu

S, D, H, DH, NSEG, L, F = 2048, 1024, 32, 32, 4, 512, 3584
G = D // 128
EPS = 1e-5
LOG2E = float(np.log2(np.e))
QSCALE = float(DH ** -0.5) * LOG2E
NEG = -1e9 * LOG2E
GELU_C = float(np.sqrt(2.0 / np.pi))
PAD = 8
MC = 128
TM4 = 2048
TMKV = 2048
ORDER = 1
SKEW = 0
UPD_POS = 1
OC = 256
FC = 512
NFC = F // FC
OFF = (0, 128, 384, 768)
TILES = tuple((j, kb) for j in range(4) for kb in range(j + 1))

PROFILE = False


def _scope(name):
    return jax.named_scope(name) if PROFILE else contextlib.nullcontext()


F32 = jnp.float32
BF16 = jnp.bfloat16
NT = (((1,), (1,)), ((), ()))


def _ln(x):
    m = jnp.mean(x, axis=-1, keepdims=True)
    d = x - m
    v = jnp.mean(d * d, axis=-1, keepdims=True)
    return d * lax.rsqrt(v + EPS)


def _gelu(x):
    return 0.5 * x * (1.0 + jnp.tanh(GELU_C * (x + 0.044715 * (x * x * x))))


def _phi(t):
    return jnp.where(t > 0, t + 1.0, jnp.exp(t))


def _dot(a, b):
    return jnp.dot(a, b, preferred_element_type=F32)


def _dot_nt(a, b):
    return lax.dot_general(a, b, NT, preferred_element_type=F32)


def _kernel(x_hbm, wq_hbm, wk_hbm, wv_hbm, wo_hbm, beta_ref, w1_hbm, w2_hbm, w3_hbm, w4_hbm,
            out_hbm,
            wq, wk, wv, wo, w1, w2, w3, w4,
            xb, xf, qs, ks, vt, pq, pk, osc, hpad, ysc, gsc, usc, msc,
            s_a, s_b, m_a, m_b, s_c, s_d, m_c, m_d, t_a, t_b, t_c, t_d, bsc, xa, xc, sems, osems, w3sems, xsems):
    TM = 512
    NT_ = S // TM

    xcps = [pltpu.make_async_copy(x_hbm.at[pl.ds(i * TM, TM), :], xb.at[pl.ds(i * TM, TM), :], xsems.at[i])
            for i in range(NT_)]
    wcps = [
        pltpu.make_async_copy(wq_hbm, wq, sems.at[0]),
        pltpu.make_async_copy(wk_hbm, wk, sems.at[1]),
        pltpu.make_async_copy(wv_hbm, wv, sems.at[2]),
        pltpu.make_async_copy(wo_hbm, wo, sems.at[3]),
        pltpu.make_async_copy(w1_hbm, w1, sems.at[4]),
        pltpu.make_async_copy(w2_hbm, w2, sems.at[5]),
        pltpu.make_async_copy(w4_hbm, w4, sems.at[6]),
    ]
    w3cps = [pltpu.make_async_copy(w3_hbm.at[:, pl.ds(n * FC, FC)], w3.at[n], w3sems.at[n]) for n in range(NFC)]
    xcps[0].start()
    wcps[0].start()

    b = beta_ref[...].astype(F32)
    gv = 1.0 / (1.0 + jnp.exp(-b))
    gb = jnp.broadcast_to(gv, (H, H))
    ri = lax.broadcasted_iota(jnp.int32, (H, H), 0)
    ci = lax.broadcasted_iota(jnp.int32, (H, H), 1)
    gcol = jnp.sum(jnp.where(ri == ci, gb, 0.0), axis=1, keepdims=True)
    gsc[...] = jnp.broadcast_to(gcol, (H, 128))

    for g in range(G):
        hpad[g, pl.ds(0, PAD), :] = jnp.zeros((PAD, 128), F32)
        hpad[g, pl.ds(PAD + S, PAD), :] = jnp.zeros((PAD, 128), F32)

    def trows(i, n=TM):
        return pl.ds(pl.multiple_of(i * TM, TM), n)

    def xcur(rows, first):
        return jnp.where(first, xb[rows, :].astype(F32), xf[rows, :])

    def stage1(first):
        @pl.when(first)
        def _():
            with _scope("xwait"):
                xcps[0].wait()
                wcps[0].wait()
            for c_ in (xcps[1], xcps[2], xcps[3], wcps[1]):
                c_.start()

        def qloop(i, c):
            @pl.when(first & (i >= 1))
            def _():
                pltpu.make_async_copy(x_hbm.at[trows(i), :], xb.at[trows(i), :], xsems.at[i]).wait()
            for mc in range(TM // MC):
                rows = pl.ds(pl.multiple_of(i * TM + mc * MC, MC), MC)
                x = _ln(xcur(rows, first)).astype(BF16)
                xa[rows, :] = x
                q = _dot(x, wq[...])
                qq = (q * QSCALE).astype(BF16)
                ph = _phi(q).astype(BF16)
                for t in range(G):
                    qs[t, rows, :] = qq[:, t * 128:(t + 1) * 128]
                    pq[t, rows, :] = ph[:, t * 128:(t + 1) * 128]
            return c
        lax.fori_loop(0, NT_, qloop, 0)

        @pl.when(first)
        def _():
            for c_ in (wcps[2], wcps[3], wcps[4]):
                c_.start()
            wcps[1].wait()

        def kloop(i, c):
            rows = pl.ds(pl.multiple_of(i * TMKV, TMKV), TMKV)
            x = xa[rows, :]
            for n in range(G // 2):
                k = _dot(x, wk[:, n * 256:(n + 1) * 256])
                kk = k.astype(BF16)
                ph = _phi(k).astype(BF16)
                for t in range(2):
                    ks[2 * n + t, rows, :] = kk[:, t * 128:(t + 1) * 128]
                    pk[2 * n + t, rows, :] = ph[:, t * 128:(t + 1) * 128]
            return c
        lax.fori_loop(0, S // TMKV, kloop, 0)

        @pl.when(first)
        def _():
            for c_ in (wcps[5],) + tuple(w3cps) + (wcps[6],):
                c_.start()
            wcps[2].wait()

        def vloop(i, c):
            x = xa[pl.ds(pl.multiple_of(i * TMKV, TMKV), TMKV), :]
            for n in range(G // 2):
                v = _dot(x, wv[:, n * 256:(n + 1) * 256])
                for t in range(2):
                    for sg in range(TMKV // L):
                        vt[2 * n + t, i * (TMKV // L) + sg, :, :] = jnp.transpose(
                            v[sg * L:(sg + 1) * L, t * 128:(t + 1) * 128]).astype(BF16)
            return c
        lax.fori_loop(0, S // TMKV, vloop, 0)

    lane = lax.broadcasted_iota(jnp.int32, (128, 128), 1)
    row = lax.broadcasted_iota(jnp.int32, (128, 128), 0)
    bsc[...] = jnp.where(row > lane, NEG, 0.0)
    NU = G * NSEG

    def step_qk(u, j, kb, s_scr, m_scr, st):
        s = u // G
        g = u % G
        r0 = pl.multiple_of(s * L, L)
        if kb == 0:
            lane64 = lax.broadcasted_iota(jnp.int32, (64, 128), 1)
            qi = pltpu.bitcast(qs[g, pl.ds(r0 + j * 128, 128), :], jnp.int32)
            st["q"] = jnp.concatenate(
                [pltpu.bitcast(jnp.where((lane64 // DH) == h, qi, 0), BF16) for h in range(4)], axis=0)
            st["mx"] = [None] * 4
        sq = _dot_nt(ks[g, pl.ds(r0 + kb * 128, 128), :], st["q"])
        o = OFF[j] + kb * 128
        for h in range(4):
            t = sq[:, h * 128:(h + 1) * 128]
            if kb == j:
                t = t + bsc[...]
            s_scr[h, o:o + 128, :] = t
            tm = jnp.max(t.reshape(16, 8, 128), axis=0)
            st["mx"][h] = tm if kb == 0 else jnp.maximum(st["mx"][h], tm)
            if kb == j:
                m_scr[j, h] = jnp.broadcast_to(jnp.max(st["mx"][h], axis=0, keepdims=True), (8, 128))

    def step_expv(u, j, kb, s_scr, m_scr, t_scr, st, use_mem):
        s = u // G
        g = u % G
        r0 = pl.multiple_of(s * L, L)
        o = OFF[j] + kb * 128
        if kb == 0:
            st["ls"] = [None] * 4
            st["acc"] = [None] * 4
            st["m"] = [m_scr[j, h] for h in range(4)]
        for h in range(4):
            t = s_scr[h, o:o + 128, :]
            p = jnp.exp2(t.reshape(16, 8, 128) - st["m"][h][None])
            ps = jnp.sum(p, axis=0)
            st["ls"][h] = ps if kb == 0 else st["ls"][h] + ps
            r = _dot(vt[g, s, pl.ds(h * DH, DH), pl.ds(kb * 128, 128)], p.reshape(128, 128).astype(BF16))
            st["acc"][h] = r if kb == 0 else st["acc"][h] + r
        if kb == j:
            if use_mem:
                nd = _dot_nt(msc[g], pq[g, pl.ds(r0 + j * 128, 128), :])
            for h in range(4):
                gh = jnp.broadcast_to(gsc[pl.ds(g * 4 + h, 1), :], (8, 128))
                l = jnp.broadcast_to(jnp.sum(st["ls"][h], axis=0, keepdims=True), (8, 128))
                cd = (1.0 - gh) / l
                acc = st["acc"][h].reshape(4, 8, 128)
                res = acc * cd[None]
                if use_mem:
                    den = jnp.broadcast_to(nd[128 + h:128 + h + 1, :], (8, 128)) + 1e-6
                    cm = gh / den
                    num = nd[h * DH:(h + 1) * DH, :].reshape(4, 8, 128)
                    res = num * cm[None] + res
                t_scr[h * DH:(h + 1) * DH, j * 128:(j + 1) * 128] = res.reshape(DH, 128)

    def mem_update(u, first):
        s = u // G
        g = u % G
        r0 = pl.multiple_of(s * L, L)
        lhs = jnp.concatenate([vt[g, s], jnp.ones((16, L), BF16)], axis=0)
        upd = _dot(lhs, pk[g, pl.ds(r0, L), :])
        r144 = lax.broadcasted_iota(jnp.int32, (144, 128), 0)
        l144 = lax.broadcasted_iota(jnp.int32, (144, 128), 1)
        rh = jnp.where(r144 < 128, r144 // DH, r144 - 128)
        acc = jnp.where(rh == l144 // DH, upd, 0.0)
        if not first:
            acc = usc[g] + acc
        usc[g] = acc
        msc[g] = acc.astype(BF16)

    def step_t(u, t_scr):
        s = u // G
        g = u % G
        r0 = pl.multiple_of(s * L, L)
        for j in range(4):
            osc[g, pl.ds(r0 + j * 128, 128), :] = jnp.transpose(t_scr[:, j * 128:(j + 1) * 128]).astype(BF16)

    def fused(u, cur, nxt, use_mem, do_upd, do_qk=True):
        a, c = {}, {}
        step_t(jnp.maximum(u - 1, 0), nxt[2])
        for (j, kb) in TILES:
            if ORDER == 0:
                step_expv(u, j, kb, cur[0], cur[1], cur[2], a, use_mem)
            if do_qk:
                step_qk(u + 1, j, kb, nxt[0], nxt[1], c)
            if ORDER == 1:
                step_expv(u, j, kb, cur[0], cur[1], cur[2], a, use_mem)
        if do_upd:
            mem_update(u, not use_mem)

    def fused2(r, cur, nxt, use_mem, do_upd, do_qk=True):
        us = (2 * r, 2 * r + 1)
        for k in range(2):
            step_t(jnp.maximum(us[k] - 2, 0), nxt[k][2])
        a, c = ({}, {}), ({}, {})
        if do_upd and UPD_POS == 0:
            for k in range(2):
                mem_update(us[k], not use_mem)
        nt = len(TILES)
        for t in range(nt + SKEW):
            for k in range(2):
                if ORDER == 0 and t < nt:
                    step_expv(us[k], *TILES[t], cur[k][0], cur[k][1], cur[k][2], a[k], use_mem)
                if do_qk and t - SKEW >= 0:
                    step_qk(us[k] + 2, *TILES[t - SKEW], nxt[k][0], nxt[k][1], c[k])
                if ORDER == 1 and t < nt:
                    step_expv(us[k], *TILES[t], cur[k][0], cur[k][1], cur[k][2], a[k], use_mem)
        if do_upd and UPD_POS == 1:
            for k in range(2):
                mem_update(us[k], not use_mem)

    def stage2(c):
        set_a = ((s_a, m_a, t_a), (s_c, m_c, t_c))
        set_b = ((s_b, m_b, t_b), (s_d, m_d, t_d))
        t_b[...] = jnp.zeros(t_b.shape, F32)
        t_d[...] = jnp.zeros(t_d.shape, F32)
        st = {}
        for k in range(2):
            for (j, kb) in TILES:
                step_qk(k, j, kb, set_a[k][0], set_a[k][1], st)

        def run(lo, hi, use_mem, do_upd):
            def one(r, c):
                @pl.when(r % 2 == 0)
                def _():
                    fused2(r, set_a, set_b, use_mem, do_upd)

                @pl.when(r % 2 == 1)
                def _():
                    fused2(r, set_b, set_a, use_mem, do_upd)
                return c
            lax.fori_loop(lo, hi, one, 0)
        NR = NU // 2
        run(0, G // 2, False, True)
        run(G // 2, NR - G // 2, True, True)
        run(NR - G // 2, NR - 1, True, False)
        fused2(NR - 1, set_b, set_a, True, False, do_qk=False)
        step_t(NU - 2, t_b)
        step_t(NU - 1, t_d)

    def stage3(first):
        def body(i, c):
            yns = []
            for mc in range(TM // MC):
                rows = pl.ds(pl.multiple_of(i * TM + mc * MC, MC), MC)
                o = jnp.concatenate([osc[g, rows, :] for g in range(G)], axis=1)
                x = xcur(rows, first) + _dot(o, wo[...])
                xf[rows, :] = x
                y = _ln(x)
                ysc[rows, :] = y
                yns.append(_ln(y).astype(BF16))
            for mc in range(TM // MC):
                r0 = pl.multiple_of(i * TM + mc * MC, MC)
                hh = _gelu(_dot(yns[mc], w1[...]))
                for t in range(G):
                    hpad[t, pl.ds(PAD + r0, MC), :] = hh[:, t * 128:(t + 1) * 128]
            return c
        lax.fori_loop(0, NT_, body, 0)

    offs = (-1, -1, 1, 1, -2, -2, 2, 2)

    def out_copy(k):
        r = pl.ds(pl.multiple_of(k * OC, OC), OC)
        return pltpu.make_async_copy(xb.at[r, :], out_hbm.at[r, :], osems.at[k])

    def stage4(last):
        def body(i, c):
            for mc in range(TM4 // MC):
                r0 = pl.multiple_of(i * TM4 + mc * MC, MC)
                rows = pl.ds(r0, MC)
                hs_in = jnp.concatenate(
                    [hpad[g, pl.ds(PAD + r0 + offs[g], MC), :] for g in range(G)], axis=1).astype(BF16)
                x1 = ysc[rows, :] + _dot(hs_in, w2[...])
                xf[rows, :] = xf[rows, :] + x1
                xc[mc * MC:(mc + 1) * MC, :] = _ln(x1).astype(BF16)
            rows = pl.ds(pl.multiple_of(i * TM4, TM4), TM4)

            def ffn(n, c):
                ub = _gelu(_dot(xc[...], w3[n])).astype(BF16)
                xf[rows, :] += _dot(ub, w4[n])
                return c
            lax.fori_loop(0, NFC - 1, ffn, 0)
            ub = _gelu(_dot(xc[...], w3[NFC - 1])).astype(BF16)
            for mc in range(TM4 // OC):
                r = pl.ds(pl.multiple_of(i * TM4 + mc * OC, OC), OC)
                xnew = xf[r, :] + _dot(ub[mc * OC:(mc + 1) * OC, :], w4[NFC - 1])
                xf[r, :] = xnew
                xb[r, :] = xnew.astype(BF16)
                out_copy(i * (TM4 // OC) + mc).start()
            return c

        @pl.when(last)
        def _():
            for k in range(S // OC):
                out_copy(k).wait()
        lax.fori_loop(0, S // TM4, body, 0)

    def layer(it, c):
        first = it == 0
        with _scope("stage1"):
            stage1(first)
        with _scope("stage2"):
            stage2(0)

        @pl.when(first)
        def _():
            wcps[3].wait()
            wcps[4].wait()
        with _scope("stage3"):
            stage3(first)

        @pl.when(first)
        def _():
            wcps[5].wait()
            for c_ in w3cps:
                c_.wait()
            wcps[6].wait()
        with _scope("stage4"):
            stage4(it == 1)
        return c

    lax.fori_loop(0, 2, layer, 0)

    for k in range(S // OC):
        out_copy(k).wait()


@jax.jit
def pallas_interleave_layers__memory_aug_infini_attn__mixer_s_mlp__prompt_kernel(
    A_x: jax.Array,
    A_wq: jax.Array,
    A_wk: jax.Array,
    A_wv: jax.Array,
    A_wo: jax.Array,
    A_beta: jax.Array,
    B_x: jax.Array,
    B_w1: jax.Array,
    B_w2: jax.Array,
    B_w3: jax.Array,
    B_w4: jax.Array,
):
    del B_x
    x = A_x.reshape(S, D)
    beta = A_beta.reshape(1, H)
    any_spec = pl.BlockSpec(memory_space=pl.ANY)
    scratch = [
        pltpu.VMEM((D, D), BF16), pltpu.VMEM((D, D), BF16), pltpu.VMEM((D, D), BF16),
        pltpu.VMEM((D, D), BF16), pltpu.VMEM((D, D), BF16), pltpu.VMEM((D, D), BF16),
        pltpu.VMEM((NFC, D, FC), BF16), pltpu.VMEM((NFC, FC, D), BF16),
        pltpu.VMEM((S, D), BF16),
        pltpu.VMEM((S, D), F32),
        pltpu.VMEM((G, S, 128), BF16),
        pltpu.VMEM((G, S, 128), BF16),
        pltpu.VMEM((G, NSEG, 128, L), BF16),
        pltpu.VMEM((G, S, 128), BF16),
        pltpu.VMEM((G, S, 128), BF16),
        pltpu.VMEM((G, S, 128), BF16),
        pltpu.VMEM((G, S + 2 * PAD, 128), F32),
        pltpu.VMEM((S, D), F32),
        pltpu.VMEM((H, 128), F32),
        pltpu.VMEM((G, 144, 128), F32),
        pltpu.VMEM((G, 144, 128), BF16),
        pltpu.VMEM((4, 1280, 128), F32), pltpu.VMEM((4, 1280, 128), F32),
        pltpu.VMEM((4, 4, 8, 128), F32), pltpu.VMEM((4, 4, 8, 128), F32),
        pltpu.VMEM((4, 1280, 128), F32), pltpu.VMEM((4, 1280, 128), F32),
        pltpu.VMEM((4, 4, 8, 128), F32), pltpu.VMEM((4, 4, 8, 128), F32),
        pltpu.VMEM((128, L), F32), pltpu.VMEM((128, L), F32),
        pltpu.VMEM((128, L), F32), pltpu.VMEM((128, L), F32),
        pltpu.VMEM((128, 128), F32),
        pltpu.VMEM((S, D), BF16), pltpu.VMEM((TM4, D), BF16),
        pltpu.SemaphoreType.DMA((7,)),
        pltpu.SemaphoreType.DMA((S // OC,)),
        pltpu.SemaphoreType.DMA((NFC,)),
        pltpu.SemaphoreType.DMA((4,)),
    ]
    out = pl.pallas_call(
        _kernel,
        out_shape=jax.ShapeDtypeStruct((S, D), BF16),
        in_specs=[any_spec] * 5 + [pl.BlockSpec(memory_space=pltpu.VMEM)] + [any_spec] * 4,
        out_specs=any_spec,
        scratch_shapes=scratch,
        compiler_params=pltpu.CompilerParams(vmem_limit_bytes=120 * 1024 * 1024),
    )(x, A_wq, A_wk, A_wv, A_wo, beta, B_w1, B_w2, B_w3, B_w4.reshape(NFC, FC, D))
    return out.reshape(1, S, D)
```

```python
import jax
import jax.numpy as jnp
import numpy as np
from jax import lax
import jax.experimental.pallas as pl
import jax.experimental.pallas.tpu as pltpu

S, D, H, DH, NSEG, L, F = 2048, 1024, 32, 32, 4, 512, 3584
G = D // 128
EPS = 1e-5
LOG2E = float(np.log2(np.e))
QSCALE = float(DH ** -0.5) * LOG2E
NEG = -1e9 * LOG2E
GELU_C = float(np.sqrt(2.0 / np.pi))
PAD = 8
MC = 128
TM4 = 2048
TMKV = 2048
OC = 256
FC = 512
NFC = F // FC
OFF = (0, 128, 384, 768)
TILES = tuple((j, kb) for j in range(4) for kb in range(j + 1))

F32 = jnp.float32
BF16 = jnp.bfloat16
NT = (((1,), (1,)), ((), ()))


def _ln(x):
    m = jnp.mean(x, axis=-1, keepdims=True)
    d = x - m
    v = jnp.mean(d * d, axis=-1, keepdims=True)
    return d * lax.rsqrt(v + EPS)


def _ln_twice(x):
    m = jnp.mean(x, axis=-1, keepdims=True)
    d = x - m
    v = jnp.mean(d * d, axis=-1, keepdims=True)
    r = lax.rsqrt(v + EPS)
    r2 = r * lax.rsqrt(v * (r * r) + EPS)
    return d * r2, m, r


def _gelu(x):
    return 0.5 * x * (1.0 + jnp.tanh(GELU_C * (x + 0.044715 * (x * x * x))))


def _phi(t):
    return jnp.where(t > 0, t + 1.0, jnp.exp(t))


def _dot(a, b):
    return jnp.dot(a, b, preferred_element_type=F32)


def _dot_nt(a, b):
    return lax.dot_general(a, b, NT, preferred_element_type=F32)


def _kernel(x_hbm, wq_hbm, wk_hbm, wv_hbm, wo_hbm, beta_ref, w1_hbm, w2_hbm, w3_hbm, w4_hbm,
            out_hbm,
            wq, wk, wv, wo, w1, w2, w3, w4,
            xb, xf, qs, ks, vt, pq, pk, osc, hpad, ysc, gsc, usc, msc,
            s_a, s_b, m_a, m_b, s_c, s_d, m_c, m_d, t_a, t_b, t_c, t_d, bsc, xa, xc, sems, osems, w3sems, xsems):
    TM = 512
    NT_ = S // TM

    xcps = [pltpu.make_async_copy(x_hbm.at[pl.ds(i * TM, TM), :], xb.at[pl.ds(i * TM, TM), :], xsems.at[i])
            for i in range(NT_)]
    wcps = [
        pltpu.make_async_copy(wq_hbm, wq, sems.at[0]),
        pltpu.make_async_copy(wk_hbm, wk, sems.at[1]),
        pltpu.make_async_copy(wv_hbm, wv, sems.at[2]),
        pltpu.make_async_copy(wo_hbm, wo, sems.at[3]),
        pltpu.make_async_copy(w1_hbm, w1, sems.at[4]),
        pltpu.make_async_copy(w2_hbm, w2, sems.at[5]),
        pltpu.make_async_copy(w4_hbm, w4, sems.at[6]),
    ]
    w3cps = [pltpu.make_async_copy(w3_hbm.at[:, pl.ds(n * FC, FC)], w3.at[n], w3sems.at[n]) for n in range(NFC)]
    xcps[0].start()
    wcps[0].start()

    b = beta_ref[...].astype(F32)
    gv = 1.0 / (1.0 + jnp.exp(-b))
    gb = jnp.broadcast_to(gv, (H, H))
    ri = lax.broadcasted_iota(jnp.int32, (H, H), 0)
    ci = lax.broadcasted_iota(jnp.int32, (H, H), 1)
    gcol = jnp.sum(jnp.where(ri == ci, gb, 0.0), axis=1, keepdims=True)
    gsc[...] = jnp.broadcast_to(gcol, (H, 128))

    for g in range(G):
        hpad[g, pl.ds(0, PAD), :] = jnp.zeros((PAD, 128), F32)
        hpad[g, pl.ds(PAD + S, PAD), :] = jnp.zeros((PAD, 128), F32)

    def trows(i, n=TM):
        return pl.ds(pl.multiple_of(i * TM, TM), n)

    def xcur(rows, first):
        return jnp.where(first, xb[rows, :].astype(F32), xf[rows, :])

    def stage1(first):
        @pl.when(first)
        def _():
            xcps[0].wait()
            wcps[0].wait()
            for c_ in (xcps[1], xcps[2], xcps[3], wcps[1]):
                c_.start()

        def qloop(i, c):
            @pl.when(first & (i >= 1))
            def _():
                pltpu.make_async_copy(x_hbm.at[trows(i), :], xb.at[trows(i), :], xsems.at[i]).wait()
            for mc in range(TM // MC):
                rows = pl.ds(pl.multiple_of(i * TM + mc * MC, MC), MC)
                x = _ln(xcur(rows, first)).astype(BF16)
                xa[rows, :] = x
                q = _dot(x, wq[...])
                qq = (q * QSCALE).astype(BF16)
                ph = _phi(q).astype(BF16)
                for t in range(G):
                    qs[t, rows, :] = qq[:, t * 128:(t + 1) * 128]
                    pq[t, rows, :] = ph[:, t * 128:(t + 1) * 128]
            return c
        lax.fori_loop(0, NT_, qloop, 0)

        @pl.when(first)
        def _():
            for c_ in (wcps[2], wcps[3], wcps[4]):
                c_.start()
            wcps[1].wait()

        def kloop(i, c):
            rows = pl.ds(pl.multiple_of(i * TMKV, TMKV), TMKV)
            x = xa[rows, :]
            for n in range(G // 2):
                k = _dot(x, wk[:, n * 256:(n + 1) * 256])
                kk = k.astype(BF16)
                ph = _phi(k).astype(BF16)
                for t in range(2):
                    ks[2 * n + t, rows, :] = kk[:, t * 128:(t + 1) * 128]
                    pk[2 * n + t, rows, :] = ph[:, t * 128:(t + 1) * 128]
            return c
        lax.fori_loop(0, S // TMKV, kloop, 0)

        @pl.when(first)
        def _():
            for c_ in (wcps[5],) + tuple(w3cps) + (wcps[6],):
                c_.start()
            wcps[2].wait()

        def vloop(i, c):
            x = xa[pl.ds(pl.multiple_of(i * TMKV, TMKV), TMKV), :]
            for n in range(G // 2):
                v = _dot(x, wv[:, n * 256:(n + 1) * 256])
                for t in range(2):
                    for sg in range(TMKV // L):
                        vt[2 * n + t, i * (TMKV // L) + sg, :, :] = jnp.transpose(
                            v[sg * L:(sg + 1) * L, t * 128:(t + 1) * 128]).astype(BF16)
            return c
        lax.fori_loop(0, S // TMKV, vloop, 0)

    lane = lax.broadcasted_iota(jnp.int32, (128, 128), 1)
    row = lax.broadcasted_iota(jnp.int32, (128, 128), 0)
    bsc[...] = jnp.where(row > lane, NEG, 0.0)
    NU = G * NSEG

    def step_qk(u, j, kb, s_scr, m_scr, st):
        s = u // G
        g = u % G
        r0 = pl.multiple_of(s * L, L)
        if kb == 0:
            lane64 = lax.broadcasted_iota(jnp.int32, (64, 128), 1)
            qi = pltpu.bitcast(qs[g, pl.ds(r0 + j * 128, 128), :], jnp.int32)
            st["q"] = jnp.concatenate(
                [pltpu.bitcast(jnp.where((lane64 // DH) == h, qi, 0), BF16) for h in range(4)], axis=0)
            st["mx"] = [None] * 4
        sq = _dot_nt(ks[g, pl.ds(r0 + kb * 128, 128), :], st["q"])
        o = OFF[j] + kb * 128
        for h in range(4):
            t = sq[:, h * 128:(h + 1) * 128]
            if kb == j:
                t = t + bsc[...]
            s_scr[h, o:o + 128, :] = t
            tm = jnp.max(t.reshape(16, 8, 128), axis=0)
            st["mx"][h] = tm if kb == 0 else jnp.maximum(st["mx"][h], tm)
            if kb == j:
                m_scr[j, h] = jnp.broadcast_to(jnp.max(st["mx"][h], axis=0, keepdims=True), (8, 128))

    def step_expv(u, j, kb, s_scr, m_scr, t_scr, st, use_mem):
        s = u // G
        g = u % G
        r0 = pl.multiple_of(s * L, L)
        o = OFF[j] + kb * 128
        if kb == 0:
            st["ls"] = [None] * 4
            st["acc"] = [None] * 4
            st["m"] = [m_scr[j, h] for h in range(4)]
        for h in range(4):
            t = s_scr[h, o:o + 128, :]
            p = jnp.exp2(t.reshape(16, 8, 128) - st["m"][h][None])
            ps = jnp.sum(p, axis=0)
            st["ls"][h] = ps if kb == 0 else st["ls"][h] + ps
            r = _dot(vt[g, s, pl.ds(h * DH, DH), pl.ds(kb * 128, 128)], p.reshape(128, 128).astype(BF16))
            st["acc"][h] = r if kb == 0 else st["acc"][h] + r
        if kb == j:
            if use_mem:
                nd = _dot_nt(msc[g], pq[g, pl.ds(r0 + j * 128, 128), :])
            for h in range(4):
                gh = jnp.broadcast_to(gsc[pl.ds(g * 4 + h, 1), :], (8, 128))
                l = jnp.broadcast_to(jnp.sum(st["ls"][h], axis=0, keepdims=True), (8, 128))
                cd = (1.0 - gh) / l
                acc = st["acc"][h].reshape(4, 8, 128)
                res = acc * cd[None]
                if use_mem:
                    den = jnp.broadcast_to(nd[128 + h:128 + h + 1, :], (8, 128)) + 1e-6
                    cm = gh / den
                    num = nd[h * DH:(h + 1) * DH, :].reshape(4, 8, 128)
                    res = num * cm[None] + res
                t_scr[h * DH:(h + 1) * DH, j * 128:(j + 1) * 128] = res.reshape(DH, 128)

    def mem_update(u, first):
        s = u // G
        g = u % G
        r0 = pl.multiple_of(s * L, L)
        lhs = jnp.concatenate([vt[g, s], jnp.ones((16, L), BF16)], axis=0)
        upd = _dot(lhs, pk[g, pl.ds(r0, L), :])
        r144 = lax.broadcasted_iota(jnp.int32, (144, 128), 0)
        l144 = lax.broadcasted_iota(jnp.int32, (144, 128), 1)
        rh = jnp.where(r144 < 128, r144 // DH, r144 - 128)
        acc = jnp.where(rh == l144 // DH, upd, 0.0)
        if not first:
            acc = usc[g] + acc
        usc[g] = acc
        msc[g] = acc.astype(BF16)

    def step_t(u, t_scr):
        s = u // G
        g = u % G
        r0 = pl.multiple_of(s * L, L)
        for j in range(4):
            osc[g, pl.ds(r0 + j * 128, 128), :] = jnp.transpose(t_scr[:, j * 128:(j + 1) * 128]).astype(BF16)

    def fused2(r, cur, nxt, use_mem, do_upd, do_qk=True):
        us = (2 * r, 2 * r + 1)
        for k in range(2):
            step_t(jnp.maximum(us[k] - 2, 0), nxt[k][2])
        a, c = ({}, {}), ({}, {})
        for tile in TILES:
            for k in range(2):
                if do_qk:
                    step_qk(us[k] + 2, *tile, nxt[k][0], nxt[k][1], c[k])
                step_expv(us[k], *tile, cur[k][0], cur[k][1], cur[k][2], a[k], use_mem)
        if do_upd:
            for k in range(2):
                mem_update(us[k], not use_mem)

    def stage2(c):
        set_a = ((s_a, m_a, t_a), (s_c, m_c, t_c))
        set_b = ((s_b, m_b, t_b), (s_d, m_d, t_d))
        t_b[...] = jnp.zeros(t_b.shape, F32)
        t_d[...] = jnp.zeros(t_d.shape, F32)
        st = {}
        for k in range(2):
            for (j, kb) in TILES:
                step_qk(k, j, kb, set_a[k][0], set_a[k][1], st)

        def run(lo, hi, use_mem, do_upd):
            def one(r, c):
                @pl.when(r % 2 == 0)
                def _():
                    fused2(r, set_a, set_b, use_mem, do_upd)

                @pl.when(r % 2 == 1)
                def _():
                    fused2(r, set_b, set_a, use_mem, do_upd)
                return c
            lax.fori_loop(lo, hi, one, 0)
        NR = NU // 2
        run(0, G // 2, False, True)
        run(G // 2, NR - G // 2, True, True)
        run(NR - G // 2, NR - 1, True, False)
        fused2(NR - 1, set_b, set_a, True, False, do_qk=False)
        step_t(NU - 2, t_b)
        step_t(NU - 1, t_d)

    def stage3(first):
        def body(i, c):
            yns = []
            for mc in range(TM // MC):
                rows = pl.ds(pl.multiple_of(i * TM + mc * MC, MC), MC)
                o = jnp.concatenate([osc[g, rows, :] for g in range(G)], axis=1)
                x = xcur(rows, first) + _dot(o, wo[...])
                xf[rows, :] = x
                yn, m, r = _ln_twice(x)
                ysc[0, rows, :] = jnp.broadcast_to(m, (MC, 128))
                ysc[1, rows, :] = jnp.broadcast_to(r, (MC, 128))
                yns.append(yn.astype(BF16))
            for mc in range(TM // MC):
                r0 = pl.multiple_of(i * TM + mc * MC, MC)
                hh = _gelu(_dot(yns[mc], w1[...]))
                for t in range(G):
                    hpad[t, pl.ds(PAD + r0, MC), :] = hh[:, t * 128:(t + 1) * 128]
            return c
        lax.fori_loop(0, NT_, body, 0)

    offs = (-1, -1, 1, 1, -2, -2, 2, 2)

    def out_copy(k):
        r = pl.ds(pl.multiple_of(k * OC, OC), OC)
        return pltpu.make_async_copy(xb.at[r, :], out_hbm.at[r, :], osems.at[k])

    def stage4(last):
        def body(i, c):
            for mc in range(TM4 // MC):
                r0 = pl.multiple_of(i * TM4 + mc * MC, MC)
                rows = pl.ds(r0, MC)
                hs_in = jnp.concatenate(
                    [hpad[g, pl.ds(PAD + r0 + offs[g], MC), :] for g in range(G)], axis=1).astype(BF16)
                x = xf[rows, :]
                y = (x - jnp.concatenate([ysc[0, rows, :]] * G, axis=1)) * jnp.concatenate([ysc[1, rows, :]] * G, axis=1)
                x1 = y + _dot(hs_in, w2[...])
                xf[rows, :] = x + x1
                xc[mc * MC:(mc + 1) * MC, :] = _ln(x1).astype(BF16)
            rows = pl.ds(pl.multiple_of(i * TM4, TM4), TM4)

            def ffn(n, c):
                ub = _gelu(_dot(xc[...], w3[n])).astype(BF16)
                xf[rows, :] += _dot(ub, w4[n])
                return c
            lax.fori_loop(0, NFC - 1, ffn, 0)
            ub = _gelu(_dot(xc[...], w3[NFC - 1])).astype(BF16)
            for mc in range(TM4 // OC):
                r = pl.ds(pl.multiple_of(i * TM4 + mc * OC, OC), OC)
                xnew = xf[r, :] + _dot(ub[mc * OC:(mc + 1) * OC, :], w4[NFC - 1])
                xf[r, :] = xnew
                xb[r, :] = xnew.astype(BF16)
                out_copy(i * (TM4 // OC) + mc).start()
            return c

        @pl.when(last)
        def _():
            for k in range(S // OC):
                out_copy(k).wait()
        lax.fori_loop(0, S // TM4, body, 0)

    def layer(it, c):
        first = it == 0
        stage1(first)
        stage2(0)

        @pl.when(first)
        def _():
            wcps[3].wait()
            wcps[4].wait()
        stage3(first)

        @pl.when(first)
        def _():
            wcps[5].wait()
            for c_ in w3cps:
                c_.wait()
            wcps[6].wait()
        stage4(it == 1)
        return c

    lax.fori_loop(0, 2, layer, 0)

    for k in range(S // OC):
        out_copy(k).wait()


@jax.jit
def pallas_interleave_layers__memory_aug_infini_attn__mixer_s_mlp__prompt_kernel(
    A_x: jax.Array,
    A_wq: jax.Array,
    A_wk: jax.Array,
    A_wv: jax.Array,
    A_wo: jax.Array,
    A_beta: jax.Array,
    B_x: jax.Array,
    B_w1: jax.Array,
    B_w2: jax.Array,
    B_w3: jax.Array,
    B_w4: jax.Array,
):
    del B_x
    x = A_x.reshape(S, D)
    beta = A_beta.reshape(1, H)
    any_spec = pl.BlockSpec(memory_space=pl.ANY)
    scratch = [
        pltpu.VMEM((D, D), BF16), pltpu.VMEM((D, D), BF16), pltpu.VMEM((D, D), BF16),
        pltpu.VMEM((D, D), BF16), pltpu.VMEM((D, D), BF16), pltpu.VMEM((D, D), BF16),
        pltpu.VMEM((NFC, D, FC), BF16), pltpu.VMEM((NFC, FC, D), BF16),
        pltpu.VMEM((S, D), BF16),
        pltpu.VMEM((S, D), F32),
        pltpu.VMEM((G, S, 128), BF16),
        pltpu.VMEM((G, S, 128), BF16),
        pltpu.VMEM((G, NSEG, 128, L), BF16),
        pltpu.VMEM((G, S, 128), BF16),
        pltpu.VMEM((G, S, 128), BF16),
        pltpu.VMEM((G, S, 128), BF16),
        pltpu.VMEM((G, S + 2 * PAD, 128), F32),
        pltpu.VMEM((2, S, 128), F32),
        pltpu.VMEM((H, 128), F32),
        pltpu.VMEM((G, 144, 128), F32),
        pltpu.VMEM((G, 144, 128), BF16),
        pltpu.VMEM((4, 1280, 128), F32), pltpu.VMEM((4, 1280, 128), F32),
        pltpu.VMEM((4, 4, 8, 128), F32), pltpu.VMEM((4, 4, 8, 128), F32),
        pltpu.VMEM((4, 1280, 128), F32), pltpu.VMEM((4, 1280, 128), F32),
        pltpu.VMEM((4, 4, 8, 128), F32), pltpu.VMEM((4, 4, 8, 128), F32),
        pltpu.VMEM((128, L), F32), pltpu.VMEM((128, L), F32),
        pltpu.VMEM((128, L), F32), pltpu.VMEM((128, L), F32),
        pltpu.VMEM((128, 128), F32),
        pltpu.VMEM((S, D), BF16), pltpu.VMEM((TM4, D), BF16),
        pltpu.SemaphoreType.DMA((7,)),
        pltpu.SemaphoreType.DMA((S // OC,)),
        pltpu.SemaphoreType.DMA((NFC,)),
        pltpu.SemaphoreType.DMA((4,)),
    ]
    out = pl.pallas_call(
        _kernel,
        out_shape=jax.ShapeDtypeStruct((S, D), BF16),
        in_specs=[any_spec] * 5 + [pl.BlockSpec(memory_space=pltpu.VMEM)] + [any_spec] * 4,
        out_specs=any_spec,
        scratch_shapes=scratch,
        compiler_params=pltpu.CompilerParams(vmem_limit_bytes=120 * 1024 * 1024),
    )(x, A_wq, A_wk, A_wv, A_wo, beta, B_w1, B_w2, B_w3, B_w4.reshape(NFC, FC, D))
    return out.reshape(1, S, D)
```
